```python
import os as _os
_os.environ.setdefault("JAX_PLATFORMS", "cpu")
import jax
import jax.numpy as jnp

def _softmax(x, axis=-1):
    return jax.nn.softmax(x, axis=axis)
def _gelu(x):
    return jax.nn.gelu(x, approximate=True)
def _silu(x):
    return jax.nn.silu(x)
def _sigmoid(x):
    return jax.nn.sigmoid(x)
def _layernorm(x, axis=-1, eps=1e-5):
    m = jnp.mean(x, axis=axis, keepdims=True)
    v = jnp.var(x, axis=axis, keepdims=True)
    return (x - m) / jnp.sqrt(v + eps)
def _scatter_add(tgt, idx, src, axis=0):
    return tgt.at[idx].add(src)
def _segment_sum(src, seg, n):
    return jax.ops.segment_sum(src, seg, n)
class _Rng:
    def __init__(self, key):
        self._k = key
    def _next(self):
        self._k, sub = jax.random.split(self._k)
        return sub
    def normal(self, shape):
        return jax.random.normal(self._next(), shape, dtype=jnp.bfloat16)
    def randint(self, lo, hi, shape):
        return jax.random.randint(self._next(), shape, lo, hi, dtype=jnp.int32)
    def uniform(self, shape, lo=0.0, hi=1.0):
        return jax.random.uniform(self._next(), shape, jnp.bfloat16, lo, hi)
    def permutation(self, n):
        return jax.random.permutation(self._next(), n)


kernel_name = 'parallel_sum__ssm_conv_h3__dense_activation_silu__prompt'

def setup_inputs():
    _rng = _Rng(jax.random.key(int.from_bytes(__import__("os").urandom(4), "little")))
    _w = (lambda a: (lambda t: t.astype(jnp.bfloat16) if jnp.issubdtype(t.dtype, jnp.floating) else t)(jnp.asarray(a)))
    def _A_setup():
        B, S, D = 1, 2048, 448
        ks = 4
        return {
            "q": _w((lambda *s: _rng.normal(s) * 0.05)(B, S, D)),
            "k": _w((lambda *s: _rng.normal(s) * 0.2)(B, S, D)),
            "v": _w((lambda *s: _rng.normal(s) * 0.2)(B, S, D)),
            "shift_k": _w((lambda *s: _rng.normal(s) * 0.2)(D, ks) * 0.5),
            "ssm_k": _w((lambda *s: _rng.normal(s) * 0.2)(D, S) * (1.0 / S ** 0.5)),
            "ssm_D": _w((lambda *s: _rng.normal(s) * 0.2)(D)),
        }
    _A_in = _A_setup()

    def _B_setup():
        B, S, D, F = 1, 2048, 448, 1792
        return {
            "x": _w((lambda *s: _rng.normal(s) * 0.05)(B, S, D)),
            "w1": _w((lambda *s: _rng.normal(s) * 0.05)(D, F) * (D ** -0.5)),
            "w2": _w((lambda *s: _rng.normal(s) * 0.05)(F, D) * (F ** -0.5)),
        }
    _B_in = _B_setup()

    return {
        "A_q": _A_in["q"],
        "A_k": _A_in["k"],
        "A_v": _A_in["v"],
        "A_shift_k": _A_in["shift_k"],
        "A_ssm_k": _A_in["ssm_k"],
        "A_ssm_D": _A_in["ssm_D"],
        "B_x": _B_in["x"],
        "B_w1": _B_in["w1"],
        "B_w2": _B_in["w2"],
    }

def reference(A_q, A_k, A_v, A_shift_k, A_ssm_k, A_ssm_D, B_x, B_w1, B_w2):
    def _A_ref(q, k, v, shift_k, ssm_k, ssm_D):
        B, S, D = q.shape
        ks = shift_k.shape[-1]
        k_pad = jnp.pad(k, ((0, 0), (ks - 1, 0), (0, 0)))
        k_shift = jnp.zeros_like(k)
        for t in range(ks):
            k_shift = k_shift + k_pad[:, t:t + S, :] * shift_k[:, ks - 1 - t][None, None, :]
        kv = k_shift * v
        L = 2 * S
        kv_pad = jnp.pad(kv, ((0, 0), (0, S), (0, 0)))
        kf_pad = jnp.pad(ssm_k, ((0, 0), (0, S)))
        kv_f = (lambda x, axes=(-2,-1): jnp.fft.rfft2(x.astype(jnp.float32), axes=axes))(kv_pad[:, None, :, :], axes=(1, 2))
        kf_f = (lambda x, axes=(-2,-1): jnp.fft.rfft2(x.astype(jnp.float32), axes=axes))(kf_pad[:, None, :], axes=(1, 2))
        kf_f = (lambda x, *d: x.transpose(*d))(kf_f, 1, 2, 0)
        y_f = kv_f * kf_f[None, :, :, :]
        y = (lambda x, s, axes=(-2,-1): jnp.fft.irfft2(x, s=s, axes=axes).astype(jnp.bfloat16))(y_f, (1, L), axes=(1, 2))[:, 0, :S, :]
        y = y + kv * ssm_D[None, None, :]
        return q * y

    def _B_ref(x, w1, w2):
        h = jnp.einsum("bsd,df->bsf", x, w1)
        h = _silu(h)
        out = jnp.einsum("bsf,fd->bsd", h, w2)
        return out

    x = A_q
    xn = _layernorm(x, axis=-1)
    return x + _A_ref(xn, A_k, A_v, A_shift_k, A_ssm_k, A_ssm_D) + _B_ref(xn, B_w1, B_w2)
```

```python
import numpy as np
import jax
import jax.numpy as jnp
import jax.experimental.pallas as pl
import jax.experimental.pallas.tpu as pltpu

S = 2048
L = 2 * S
N1 = 64
N2 = 64
NZ = S // N2
K2P = 40
RB = 256


def _consts():
    n1 = np.arange(NZ)[None, None, :]
    n2 = np.arange(N2)[:, None, None]
    k1 = np.arange(N1)[None, :, None]
    th = 2 * np.pi * ((64 * n1 + n2) * k1 % L) / L
    G = np.concatenate([np.cos(th), -np.sin(th)], axis=1)
    H = np.concatenate([np.cos(th), -np.sin(th)], axis=1).transpose(0, 2, 1) / L
    k2 = np.arange(K2P)[:, None]
    m2 = np.arange(N2)[None, :]
    ph = 2 * np.pi * (k2 * m2 % N2) / N2
    C, Sn = np.cos(ph), np.sin(ph)
    F2 = np.block([[C, Sn], [-Sn, C]])
    IFs = []
    for first in (True, False):
        a = np.zeros(K2P)
        a[:32] = 2.0
        if first:
            a[0] = 1.0
            a[32] = 1.0
        Ca, Sa = (C * a[:, None]).T, (Sn * a[:, None]).T
        IFs.append(np.block([[Ca, -Sa], [Sa, Ca]]))
    IF2 = np.stack(IFs)
    f = lambda a: jnp.asarray(a, dtype=jnp.bfloat16)
    return f(G), f(F2), f(IF2), f(H)


def _kernel(q_ref, k_ref, v_ref, sk_ref, kt_ref, d_ref, w1_ref, w2_ref,
            g_ref, f2_ref, if2_ref, h_ref, o_ref,
            kv_s, kt_s, zx_s, zk_s):
    f32, bf16 = jnp.float32, jnp.bfloat16
    D = q_ref.shape[-1]

    k = k_ref[...].astype(f32)
    sk = sk_ref[...].astype(f32)
    row = jax.lax.broadcasted_iota(jnp.int32, (S, D), 0)
    ks = k * sk[0:1, :]
    for j in range(1, 4):
        kj = jnp.where(row >= j, pltpu.roll(k, j, 0), 0.0)
        ks = ks + kj * sk[j:j + 1, :]
    kv = ks * v_ref[...].astype(f32)
    kt = kt_ref[...].astype(f32)
    dv = d_ref[...].astype(f32)
    NT = kv_s.shape[0]
    for j in range(NT):
        w = min(128, D - 128 * j)
        if w < 128:
            kv_s[j] = jnp.zeros((S, 128), f32)
            kt_s[j] = jnp.zeros((S, 128), f32)
        kv_s[j, :, :w] = kv[:, 128 * j:128 * j + w]
        kt_s[j, :, :w] = kt[:, 128 * j:128 * j + w]

    def loop_a(n2, _):
        g = g_ref[n2]
        for src, dst in ((kv_s, zx_s), (kt_s, zk_s)):
            for j in range(NT):
                xs = src[j, pl.ds(n2, NZ, stride=N2), :].astype(bf16)
                z = jnp.dot(g, xs, preferred_element_type=f32)
                dst[j, pl.ds(n2, N1, stride=128), :] = z[:N1]
                dst[j, pl.ds(N2 + n2, N1, stride=128), :] = z[N1:]
        return 0
    jax.lax.fori_loop(0, N2, loop_a, 0)

    def loop_b(k1, _):
        r = pl.multiple_of(k1 * 128, 128)
        f2 = f2_ref[...]
        if2 = if2_ref[jnp.minimum(k1, 1)]
        for j in range(NT):
            xf = jnp.dot(f2, zx_s[j, pl.ds(r, 128), :].astype(bf16), preferred_element_type=f32)
            kf = jnp.dot(f2, zk_s[j, pl.ds(r, 128), :].astype(bf16), preferred_element_type=f32)
            xr, xi, kr, ki = xf[:K2P], xf[K2P:], kf[:K2P], kf[K2P:]
            y = jnp.concatenate([xr * kr - xi * ki, xr * ki + xi * kr], axis=0).astype(bf16)
            zx_s[j, pl.ds(r, 128), :] = jnp.dot(if2, y, preferred_element_type=f32)
        return 0
    jax.lax.fori_loop(0, N1, loop_b, 0)

    def loop_c(n2, _):
        hm = h_ref[n2]
        for j in range(NT):
            u = jnp.concatenate([zx_s[j, pl.ds(n2, N1, stride=128), :],
                                 zx_s[j, pl.ds(N2 + n2, N1, stride=128), :]], axis=0).astype(bf16)
            kt_s[j, pl.ds(n2, NZ, stride=N2), :] = jnp.dot(hm, u, preferred_element_type=f32)
        return 0
    jax.lax.fori_loop(0, N2, loop_c, 0)

    def loop_d(i, _):
        r = pl.multiple_of(i * RB, RB)
        x = q_ref[pl.ds(r, RB), :].astype(f32)
        m = jnp.mean(x, axis=-1, keepdims=True)
        xc = x - m
        var = jnp.mean(xc * xc, axis=-1, keepdims=True)
        xn = xc * jax.lax.rsqrt(var + 1e-5)
        h = jnp.dot(xn.astype(bf16), w1_ref[...], preferred_element_type=f32)
        h = (h * jax.nn.sigmoid(h)).astype(bf16)
        mlp = jnp.dot(h, w2_ref[...], preferred_element_type=f32)
        cat = lambda ref: jnp.concatenate([ref[j, pl.ds(r, RB), :] for j in range(NT)], axis=1)[:, :D]
        yt = cat(kt_s) + cat(kv_s) * dv
        o_ref[pl.ds(r, RB), :] = (x + xn * yt + mlp).astype(o_ref.dtype)
        return 0
    jax.lax.fori_loop(0, S // RB, loop_d, 0)


@jax.jit
def pallas_parallel_sum__ssm_conv_h3__dense_activation_silu__prompt_kernel(
    A_q, A_k, A_v, A_shift_k, A_ssm_k, A_ssm_D, B_x, B_w1, B_w2):
    _, s, d = A_q.shape
    nt = -(-d // 128)
    G, F2, IF2, H = _consts()
    out = pl.pallas_call(
        _kernel,
        out_shape=jax.ShapeDtypeStruct((s, d), A_q.dtype),
        scratch_shapes=[
            pltpu.VMEM((nt, s, 128), jnp.float32),
            pltpu.VMEM((nt, s, 128), jnp.float32),
            pltpu.VMEM((nt, N1 * 128, 128), jnp.float32),
            pltpu.VMEM((nt, N1 * 128, 128), jnp.float32),
        ],
        compiler_params=pltpu.CompilerParams(vmem_limit_bytes=100 * 1024 * 1024),
    )(A_q[0], A_k[0], A_v[0], A_shift_k.T, A_ssm_k.T, A_ssm_D[None, :], B_w1, B_w2,
      G, F2, IF2, H)
    return out[None]
```

```python
import numpy as np
import jax
import jax.numpy as jnp
import jax.experimental.pallas as pl
import jax.experimental.pallas.tpu as pltpu

S = 2048
L = 2 * S
N1 = 64
N2 = 64
NZ = S // N2
K1P = 40
RB = 256


def _consts():
    n1 = np.arange(NZ)[None, None, :]
    n2 = np.arange(N2)[:, None, None]
    k1 = np.arange(K1P)[None, :, None]
    th = 2 * np.pi * ((64 * n1 + n2) * k1 % L) / L
    valid = (np.arange(K1P) <= 32).astype(np.float64)[None, :, None]
    wt = np.where((np.arange(K1P) == 0) | (np.arange(K1P) == 32), 1.0, 2.0)[None, :, None] * valid
    G = np.concatenate([np.cos(th) * valid, -np.sin(th) * valid], axis=1)
    H = np.concatenate([np.cos(th) * wt, -np.sin(th) * wt], axis=1).transpose(0, 2, 1) / L
    k2 = np.arange(N2)[:, None]
    m2 = np.arange(N2)[None, :]
    ph = 2 * np.pi * (k2 * m2 % N2) / N2
    C, Sn = np.cos(ph), np.sin(ph)
    F2 = np.block([[C, Sn], [-Sn, C]])
    IF2 = np.block([[C, -Sn], [Sn, C]])
    f = lambda a: jnp.asarray(a, dtype=jnp.bfloat16)
    return f(G), f(F2), f(IF2), f(H)


def _kernel(q_hbm, k_ref, v_ref, sk_ref, kt_ref, d_ref, w1_hbm, w2_hbm,
            g_ref, f2_ref, if2_ref, h_ref, o_ref,
            kv_s, kt_s, zx_s, zk_s, q_ref, w1_ref, w2_ref, sems):
    cps = [pltpu.make_async_copy(a, b, sems.at[i]) for i, (a, b) in
           enumerate(((q_hbm, q_ref), (w1_hbm, w1_ref), (w2_hbm, w2_ref)))]
    for c in cps:
        c.start()
    f32, bf16 = jnp.float32, jnp.bfloat16
    D = q_ref.shape[0]

    k = k_ref[...].astype(f32).T
    sk = sk_ref[...].astype(f32)
    row = jax.lax.broadcasted_iota(jnp.int32, (S, D), 0)
    ks = k * sk[0:1, :]
    for j in range(1, 4):
        kj = jnp.where(row >= j, pltpu.roll(k, j, 0), 0.0)
        ks = ks + kj * sk[j:j + 1, :]
    kv = ks * v_ref[...].astype(f32).T
    kt = kt_ref[...].astype(f32).T
    dv = d_ref[...].astype(f32)
    NT = kv_s.shape[0]
    for j in range(NT):
        w = min(128, D - 128 * j)
        if w < 128:
            kv_s[j] = jnp.zeros((S, 128), f32)
            kt_s[j] = jnp.zeros((S, 128), f32)
        kv_s[j, :, :w] = kv[:, 128 * j:128 * j + w]
        kt_s[j, :, :w] = kt[:, 128 * j:128 * j + w]

    def loop_a(n2, _):
        g = g_ref[n2]
        for src, dst in ((kv_s, zx_s), (kt_s, zk_s)):
            for j in range(NT):
                xs = src[j, pl.ds(n2, NZ, stride=N2), :].astype(bf16)
                z = jnp.dot(g, xs, preferred_element_type=f32)
                dst[j, pl.ds(n2, K1P, stride=128), :] = z[:K1P]
                dst[j, pl.ds(N2 + n2, K1P, stride=128), :] = z[K1P:]
        return 0
    jax.lax.fori_loop(0, N2, loop_a, 0, unroll=8)

    def loop_b(k1, _):
        r = pl.multiple_of(k1 * 128, 128)
        f2 = f2_ref[...]
        if2 = if2_ref[...]
        for j in range(NT):
            xf = jnp.dot(f2, zx_s[j, pl.ds(r, 128), :].astype(bf16), preferred_element_type=f32)
            kf = jnp.dot(f2, zk_s[j, pl.ds(r, 128), :].astype(bf16), preferred_element_type=f32)
            xr, xi, kr, ki = xf[:N2], xf[N2:], kf[:N2], kf[N2:]
            y = jnp.concatenate([xr * kr - xi * ki, xr * ki + xi * kr], axis=0).astype(bf16)
            zx_s[j, pl.ds(r, 128), :] = jnp.dot(if2, y, preferred_element_type=f32)
        return 0
    jax.lax.fori_loop(0, 33, loop_b, 0, unroll=3)

    def loop_c(n2, _):
        hm = h_ref[n2]
        for j in range(NT):
            u = jnp.concatenate([zx_s[j, pl.ds(n2, K1P, stride=128), :],
                                 zx_s[j, pl.ds(N2 + n2, K1P, stride=128), :]], axis=0).astype(bf16)
            kt_s[j, pl.ds(n2, NZ, stride=N2), :] = jnp.dot(hm, u, preferred_element_type=f32)
        return 0
    jax.lax.fori_loop(0, N2, loop_c, 0, unroll=8)

    for c in cps:
        c.wait()

    def loop_d(i, _):
        r = pl.multiple_of(i * RB, RB)
        x = q_ref[:, pl.ds(r, RB)].astype(f32)
        m = jnp.mean(x, axis=0, keepdims=True)
        xc = x - m
        var = jnp.mean(xc * xc, axis=0, keepdims=True)
        xn = xc * jax.lax.rsqrt(var + 1e-5)
        h = jax.lax.dot_general(w1_ref[...], xn.astype(bf16), (((0,), (0,)), ((), ())),
                                preferred_element_type=f32)
        h = (h * jax.nn.sigmoid(h)).astype(bf16)
        mlp = jnp.dot(w2_ref[...], h, preferred_element_type=f32)
        cat = lambda ref: jnp.concatenate([ref[j, pl.ds(r, RB), :] for j in range(NT)], axis=1)[:, :D]
        yt = (cat(kt_s) + cat(kv_s) * dv).T
        o_ref[:, pl.ds(r, RB)] = (x + xn * yt + mlp).astype(o_ref.dtype)
        return 0
    jax.lax.fori_loop(0, S // RB, loop_d, 0)


@jax.jit
def pallas_parallel_sum__ssm_conv_h3__dense_activation_silu__prompt_kernel(
    A_q, A_k, A_v, A_shift_k, A_ssm_k, A_ssm_D, B_x, B_w1, B_w2):
    _, s, d = A_q.shape
    nt = -(-d // 128)
    G, F2, IF2, H = _consts()
    out = pl.pallas_call(
        _kernel,
        out_shape=jax.ShapeDtypeStruct((d, s), A_q.dtype),
        scratch_shapes=[
            pltpu.VMEM((nt, s, 128), jnp.float32),
            pltpu.VMEM((nt, s, 128), jnp.float32),
            pltpu.VMEM((nt, K1P * 128, 128), jnp.float32),
            pltpu.VMEM((nt, K1P * 128, 128), jnp.float32),
            pltpu.VMEM((d, s), jnp.bfloat16),
            pltpu.VMEM(B_w1.shape, jnp.bfloat16),
            pltpu.VMEM(B_w2.shape[::-1], jnp.bfloat16),
            pltpu.SemaphoreType.DMA((3,)),
        ],
        in_specs=[pl.BlockSpec(memory_space=pl.ANY if i in (0, 6, 7) else pltpu.VMEM) for i in range(12)],
        compiler_params=pltpu.CompilerParams(vmem_limit_bytes=100 * 1024 * 1024),
    )(A_q[0].T, A_k[0].T, A_v[0].T, A_shift_k.T, A_ssm_k, A_ssm_D[None, :], B_w1, B_w2.T,
      G, F2, IF2, H)
    return out.T[None]
```
